```python
import os as _os
_os.environ.setdefault("JAX_PLATFORMS", "cpu")
import jax
import jax.numpy as jnp

def _softmax(x, axis=-1):
    return jax.nn.softmax(x, axis=axis)
def _gelu(x):
    return jax.nn.gelu(x, approximate=True)
def _silu(x):
    return jax.nn.silu(x)
def _sigmoid(x):
    return jax.nn.sigmoid(x)
def _layernorm(x, axis=-1, eps=1e-5):
    m = jnp.mean(x, axis=axis, keepdims=True)
    v = jnp.var(x, axis=axis, keepdims=True)
    return (x - m) / jnp.sqrt(v + eps)
def _scatter_add(tgt, idx, src, axis=0):
    return tgt.at[idx].add(src)
def _segment_sum(src, seg, n):
    return jax.ops.segment_sum(src, seg, n)
class _Rng:
    def __init__(self, key):
        self._k = key
    def _next(self):
        self._k, sub = jax.random.split(self._k)
        return sub
    def normal(self, shape):
        return jax.random.normal(self._next(), shape, dtype=jnp.bfloat16)
    def randint(self, lo, hi, shape):
        return jax.random.randint(self._next(), shape, lo, hi, dtype=jnp.int32)
    def uniform(self, shape, lo=0.0, hi=1.0):
        return jax.random.uniform(self._next(), shape, jnp.bfloat16, lo, hi)
    def permutation(self, n):
        return jax.random.permutation(self._next(), n)


kernel_name = 'parallel_sum__ssm_conv_s5__geglu_ffn__prompt'

def setup_inputs():
    _rng = _Rng(jax.random.key(int.from_bytes(__import__("os").urandom(4), "little")))
    _w = (lambda a: (lambda t: t.astype(jnp.bfloat16) if jnp.issubdtype(t.dtype, jnp.floating) else t)(jnp.asarray(a)))
    def _A_setup():
        B, S, D = 1, 2048, 512
        P = D
        Lambda_re = -0.5 * jnp.exp((lambda *s: _rng.normal(s) * 0.8)(P))
        Lambda_im = (lambda *s: _rng.normal(s) * 0.8)(P) * 1.0
        B_re = (lambda *s: _rng.normal(s) * 0.8)(P, D) * (D ** -0.5)
        B_im = (lambda *s: _rng.normal(s) * 0.8)(P, D) * (D ** -0.5)
        C_re = (lambda *s: _rng.normal(s) * 0.8)(D, P) * (P ** -0.5)
        C_im = (lambda *s: _rng.normal(s) * 0.8)(D, P) * (P ** -0.5)
        log_dt = (lambda *s: _rng.normal(s) * 0.8)(P) * 0.3 - 2.0
        Dskip = (lambda *s: _rng.normal(s) * 0.8)(D)
        return {
            "x": _w((lambda *s: _rng.normal(s) * 0.05)(B, S, D)),
            "Lambda_re": _w(Lambda_re),
            "Lambda_im": _w(Lambda_im),
            "B_re": _w(B_re),
            "B_im": _w(B_im),
            "C_re": _w(C_re),
            "C_im": _w(C_im),
            "log_dt": _w(log_dt),
            "Dskip": _w(Dskip),
        }
    _A_in = _A_setup()

    def _B_setup():
        B, S, D, F = 1, 2048, 512, 1376
        return {
            "x": _w((lambda *s: _rng.normal(s) * 0.05)(B, S, D)),
            "w_gate": _w((lambda *s: _rng.normal(s) * 0.05)(D, F)),
            "w_up": _w((lambda *s: _rng.normal(s) * 0.05)(D, F)),
            "w_down": _w((lambda *s: _rng.normal(s) * 0.05)(F, D)),
        }
    _B_in = _B_setup()

    return {
        "A_x": _A_in["x"],
        "A_Lambda_re": _A_in["Lambda_re"],
        "A_Lambda_im": _A_in["Lambda_im"],
        "A_B_re": _A_in["B_re"],
        "A_B_im": _A_in["B_im"],
        "A_C_re": _A_in["C_re"],
        "A_C_im": _A_in["C_im"],
        "A_log_dt": _A_in["log_dt"],
        "A_Dskip": _A_in["Dskip"],
        "B_x": _B_in["x"],
        "B_w_gate": _B_in["w_gate"],
        "B_w_up": _B_in["w_up"],
        "B_w_down": _B_in["w_down"],
    }

def reference(A_x, A_Lambda_re, A_Lambda_im, A_B_re, A_B_im, A_C_re, A_C_im, A_log_dt, A_Dskip, B_x, B_w_gate, B_w_up, B_w_down):
    def _A_ref(x, Lambda_re, Lambda_im, B_re, B_im, C_re, C_im, log_dt, Dskip):
        Bsz, L, H = x.shape
        Lam = Lambda_re + 1j * Lambda_im
        Bmat = B_re + 1j * B_im
        Cmat = C_re + 1j * C_im
        dt = jnp.exp(log_dt)
        Lam_bar = jnp.exp(dt * Lam)
        B_bar = ((Lam_bar - 1.0) / Lam)[:, None] * Bmat
        Bu = jnp.einsum("bld,pd->blp", x + 0j, B_bar)
        h = jnp.zeros_like(Bu[:, 0, :])
        hs = []
        for t in range(L):
            h = Lam_bar[None, :] * h + Bu[:, t, :]
            hs.append(h)
        hseq = jnp.stack(hs, 1)
        y = 2.0 * jnp.einsum("blp,dp->bld", hseq, Cmat).real + x * Dskip[None, None, :]
        return y

    def _B_ref(x, w_gate, w_up, w_down):
        return (_gelu(x @ w_gate) * (x @ w_up)) @ w_down

    x = A_x
    xn = _layernorm(x, axis=-1)
    return x + _A_ref(xn, A_Lambda_re, A_Lambda_im, A_B_re, A_B_im, A_C_re, A_C_im, A_log_dt, A_Dskip) + _B_ref(xn, B_w_gate, B_w_up, B_w_down)
```

```python
import functools
import jax
import jax.numpy as jnp
import jax.experimental.pallas as pl
import jax.experimental.pallas.tpu as pltpu

TC = 256
NSEG = 8
SEG = TC // NSEG + 1
LAST = TC - (NSEG - 1) * SEG
FSPLIT = 768


def _cpow(pr, pi, n):
    rr, ri = None, None
    while n:
        if n & 1:
            if rr is None:
                rr, ri = pr, pi
            else:
                rr, ri = rr * pr - ri * pi, rr * pi + ri * pr
        n >>= 1
        if n:
            pr, pi = pr * pr - pi * pi, 2.0 * pr * pi
    return rr, ri


def _kernel(x_hbm, lre_hbm, lim_hbm, ldt_hbm, dskip_hbm,
            bre_hbm, bim_hbm, cre_hbm, cim_hbm, wg_hbm, wu_hbm, wd_hbm,
            o_ref,
            lre_ref, lim_ref, ldt_ref, dskip_ref,
            bre_ref, bim_ref, cre_ref, cim_ref, wg_ref, wu_ref, wd_ref, sems, xsems,
            cst_ref, lam_ref, carry_ref, hin_ref, bu_ref, xn_ref, xbuf):
    P = bre_ref.shape[0]
    F = wg_ref.shape[0]
    f32 = jnp.float32
    bf16 = jnp.bfloat16
    NG = P // 128
    step_i = pl.program_id(0)
    nsteps = pl.num_programs(0)

    lo = lambda r: r.at[0:FSPLIT]
    hi = lambda r: r.at[FSPLIT:F]
    pairs = dict(lre=(lre_hbm, lre_ref), lim=(lim_hbm, lim_ref), ldt=(ldt_hbm, ldt_ref),
                 dskip=(dskip_hbm, dskip_ref),
                 bre=(bre_hbm, bre_ref), bim=(bim_hbm, bim_ref),
                 wg0=(lo(wg_hbm), lo(wg_ref)), wg1=(hi(wg_hbm), hi(wg_ref)),
                 wu0=(lo(wu_hbm), lo(wu_ref)), wu1=(hi(wu_hbm), hi(wu_ref)),
                 cre=(cre_hbm, cre_ref), cim=(cim_hbm, cim_ref),
                 wd=(wd_hbm, wd_ref))
    order = list(pairs)

    def copy(name):
        src, dst = pairs[name]
        return pltpu.make_async_copy(src, dst, sems.at[order.index(name)])

    def xcopy(c):
        slot = c % 3
        return pltpu.make_async_copy(x_hbm.at[pl.ds(c * TC, TC)], xbuf.at[slot], xsems.at[slot])

    def init_small():
        lre = lre_ref[...].astype(f32).reshape(1, P)
        lim = lim_ref[...].astype(f32).reshape(1, P)
        ldt = ldt_ref[...].astype(f32).reshape(1, P)
        dt = jnp.exp(ldt).astype(bf16).astype(f32)
        e = jnp.exp(dt * lre)
        lbr = e * jnp.cos(dt * lim)
        lbi = e * jnp.sin(dt * lim)
        nr = lbr - 1.0
        ni = lbi
        den = lre * lre + lim * lim
        cr = (nr * lre + ni * lim) / den
        ci = (ni * lre - nr * lim) / den
        lam_ref[0:1, :] = lbr
        lam_ref[1:2, :] = lbi
        pr, pi = _cpow(lbr, lbi, SEG)
        lam_ref[2:3, :] = pr
        lam_ref[3:4, :] = pi
        pr, pi = _cpow(lbr, lbi, LAST)
        lam_ref[4:5, :] = pr
        lam_ref[5:6, :] = pi
        lam_ref[6:7, :] = cr
        lam_ref[7:8, :] = ci
        carry_ref[...] = jnp.zeros_like(carry_ref)
        for g in range(2 * NG):
            bu_ref[g, TC:NSEG * SEG, :] = jnp.zeros((NSEG * SEG - TC, 128), f32)

    def init_c():
        cr = lam_ref[6:7, :]
        ci = lam_ref[7:8, :]
        c_re = cre_ref[...].astype(f32)
        c_im = cim_ref[...].astype(f32)
        cst_ref[:, 0:P] = (2.0 * (c_re * cr - c_im * ci)).astype(bf16)
        cst_ref[:, P:2 * P] = (-2.0 * (c_re * ci + c_im * cr)).astype(bf16)

    def layernorm(ref):
        x = ref[...].astype(f32)
        m = jnp.mean(x, axis=-1, keepdims=True)
        xc = x - m
        v = jnp.mean(xc * xc, axis=-1, keepdims=True)
        return (xc * jax.lax.rsqrt(v + 1e-5)).astype(bf16)

    def body(first):
        def start(*names):
            for n in names:
                if n.startswith('x'):
                    xcopy(int(n[1:])).start()
                else:
                    copy(n).start()

        after = dict(bre=['wg0'], bim=['wu0'], wg0=['wg1'], wu0=['wu1', 'x1'], wg1=['cre', 'cim'],
                     wu1=['wd'], cre=['x2'])

        def wait(*names):
            if first:
                for n in names:
                    copy(n).wait()
                    start(*after.get(n, []))

        nt = (((1,), (1,)), ((), ()))
        if first:
            start('x0', 'bre', 'lre', 'lim', 'ldt', 'dskip')
            x_cur = xbuf.at[0]
            x_nxt = xbuf.at[1]
            xcopy(0).wait()
            start('bim')
            xn = layernorm(x_cur)
        else:
            x_cur = xbuf.at[step_i % 3]
            x_nxt = xbuf.at[(step_i + 1) % 3]

            @pl.when(step_i + 2 < nsteps)
            def _():
                xcopy(step_i + 2).start()

            @pl.when(step_i + 1 < nsteps)
            def _():
                xcopy(step_i + 1).wait()

            xn = xn_ref[...]

        wait('bre')
        bu = jax.lax.dot_general(xn, bre_ref[...], nt, preferred_element_type=f32)
        for g in range(NG):
            bu_ref[g, 0:TC, :] = bu[:, g * 128:(g + 1) * 128]
        wait('bim')
        bu = jax.lax.dot_general(xn, bim_ref[...], nt, preferred_element_type=f32)
        for g in range(NG):
            bu_ref[NG + g, 0:TC, :] = bu[:, g * 128:(g + 1) * 128]

        if first:
            wait('lre', 'lim', 'ldt', 'dskip')
            init_small()
        else:
            xn_next = layernorm(x_nxt)

        if first:
            parts = []
            for k, (a0, a1) in enumerate([(0, FSPLIT), (FSPLIT, F)]):
                wait('wg%d' % k)
                g = jax.lax.dot_general(xn, wg_ref[a0:a1, :], nt, preferred_element_type=f32)
                wait('wu%d' % k)
                u = jax.lax.dot_general(xn, wu_ref[a0:a1, :], nt, preferred_element_type=f32)
                parts.append((jax.nn.gelu(g, approximate=True) * u).astype(bf16))
            xcopy(1).wait()
            xn_next = layernorm(x_nxt)
        else:
            g = jax.lax.dot_general(xn, wg_ref[...], nt, preferred_element_type=f32)
            u = jax.lax.dot_general(xn, wu_ref[...], nt, preferred_element_type=f32)
            a = (jax.nn.gelu(g, approximate=True) * u).astype(bf16)

        lr = jnp.broadcast_to(lam_ref[0:1, :], (NSEG, P))
        li = jnp.broadcast_to(lam_ref[1:2, :], (NSEG, P))

        def step(j, h):
            hr, hi = h
            br = jnp.concatenate([bu_ref[g, pl.ds(j, NSEG, stride=SEG), :] for g in range(NG)], axis=1)
            bi = jnp.concatenate([bu_ref[NG + g, pl.ds(j, NSEG, stride=SEG), :] for g in range(NG)], axis=1)
            return lr * hr - li * hi + br, lr * hi + li * hr + bi

        z = jnp.zeros((NSEG, P), f32)
        fr, fi = jax.lax.fori_loop(0, LAST, step, (z, z), unroll=True)
        er, ei = jax.lax.fori_loop(LAST, SEG, step, (fr, fi), unroll=True)

        pr = lam_ref[2:3, :]
        pi = lam_ref[3:4, :]
        cr = carry_ref[0:1, :]
        ci = carry_ref[1:2, :]
        for s in range(NSEG):
            hin_ref[s:s + 1, 0:P] = cr
            hin_ref[s:s + 1, P:2 * P] = ci
            if s < NSEG - 1:
                cr, ci = (pr * cr - pi * ci + er[s:s + 1, :], pr * ci + pi * cr + ei[s:s + 1, :])
            else:
                pr = lam_ref[4:5, :]
                pi = lam_ref[5:6, :]
                cr, ci = (pr * cr - pi * ci + fr[s:s + 1, :], pr * ci + pi * cr + fi[s:s + 1, :])
        carry_ref[0:1, :] = cr
        carry_ref[1:2, :] = ci

        def step2(j, h):
            nr, ni = step(j, h)
            for g in range(NG):
                bu_ref[g, pl.ds(j, NSEG, stride=SEG), :] = nr[:, g * 128:(g + 1) * 128]
                bu_ref[NG + g, pl.ds(j, NSEG, stride=SEG), :] = ni[:, g * 128:(g + 1) * 128]
            return nr, ni

        h = jax.lax.fori_loop(0, LAST, step2, (hin_ref[:, 0:P], hin_ref[:, P:2 * P]), unroll=True)

        keep = jax.lax.broadcasted_iota(jnp.int32, (NSEG, P), 0) < NSEG - 1

        def step3(j, h):
            nr, ni = step(j, h)
            sr = jnp.where(keep, nr, 0.0)
            si = jnp.where(keep, ni, 0.0)
            for g in range(NG):
                bu_ref[g, pl.ds(j, NSEG, stride=SEG), :] = sr[:, g * 128:(g + 1) * 128]
                bu_ref[NG + g, pl.ds(j, NSEG, stride=SEG), :] = si[:, g * 128:(g + 1) * 128]
            return nr, ni

        jax.lax.fori_loop(LAST, SEG, step3, h, unroll=True)

        wait('cre', 'cim')
        if first:
            init_c()
        hb = jnp.concatenate([bu_ref[g, 0:TC, :] for g in range(2 * NG)], axis=1).astype(bf16)
        y = jax.lax.dot_general(hb, cst_ref[...], nt, preferred_element_type=f32)

        wait('wd')
        if first:
            ff = (jnp.dot(parts[0], wd_ref[0:FSPLIT, :], preferred_element_type=f32)
                  + jnp.dot(parts[1], wd_ref[FSPLIT:F, :], preferred_element_type=f32))
        else:
            ff = jnp.dot(a, wd_ref[...], preferred_element_type=f32)

        xn_ref[...] = xn_next
        o_ref[...] = (x_cur[...].astype(f32) + y
                      + xn.astype(f32) * dskip_ref[...].astype(f32).reshape(1, P) + ff)

    pl.when(step_i == 0)(lambda: body(True))
    pl.when(step_i != 0)(lambda: body(False))


@jax.jit
def pallas_parallel_sum__ssm_conv_s5__geglu_ffn__prompt_kernel(
    A_x, A_Lambda_re, A_Lambda_im, A_B_re, A_B_im, A_C_re, A_C_im, A_log_dt, A_Dskip,
    B_x, B_w_gate, B_w_up, B_w_down,
):
    Bsz, L, D = A_x.shape
    P = A_Lambda_re.shape[0]
    F = B_w_gate.shape[1]
    x = A_x.reshape(L, D)
    hbm = pl.BlockSpec(memory_space=pl.ANY)
    out = pl.pallas_call(
        _kernel,
        grid=(L // TC,),
        in_specs=[hbm] * 12,
        out_specs=pl.BlockSpec((TC, D), lambda i: (i, 0)),
        out_shape=jax.ShapeDtypeStruct((L, D), jnp.float32),
        scratch_shapes=[
            pltpu.VMEM((P,), jnp.bfloat16), pltpu.VMEM((P,), jnp.bfloat16),
            pltpu.VMEM((P,), jnp.bfloat16), pltpu.VMEM((D,), jnp.bfloat16),
            pltpu.VMEM((P, D), jnp.bfloat16), pltpu.VMEM((P, D), jnp.bfloat16),
            pltpu.VMEM((D, P), jnp.bfloat16), pltpu.VMEM((D, P), jnp.bfloat16),
            pltpu.VMEM((F, D), jnp.bfloat16), pltpu.VMEM((F, D), jnp.bfloat16),
            pltpu.VMEM((F, D), jnp.bfloat16),
            pltpu.SemaphoreType.DMA((13,)),
            pltpu.SemaphoreType.DMA((3,)),
            pltpu.VMEM((D, 2 * P), jnp.bfloat16),
            pltpu.VMEM((8, P), jnp.float32),
            pltpu.VMEM((8, P), jnp.float32),
            pltpu.VMEM((NSEG, 2 * P), jnp.float32),
            pltpu.VMEM((2 * P // 128, NSEG * SEG, 128), jnp.float32),
            pltpu.VMEM((TC, D), jnp.bfloat16),
            pltpu.VMEM((3, TC, D), jnp.bfloat16),
        ],
        compiler_params=pltpu.CompilerParams(
            dimension_semantics=("arbitrary",),
            vmem_limit_bytes=96 * 1024 * 1024,
        ),
    )(x, A_Lambda_re, A_Lambda_im, A_log_dt, A_Dskip,
      A_B_re, A_B_im, A_C_re, A_C_im, B_w_gate.T, B_w_up.T, B_w_down)
    return out.reshape(Bsz, L, D)
```

```python
import jax
import jax.numpy as jnp
import jax.experimental.pallas as pl
import jax.experimental.pallas.tpu as pltpu

TC = 256
NSEG = 8
SEG = TC // NSEG + 1
LAST = TC - (NSEG - 1) * SEG
FSPLIT = 768


def _cpow(pr, pi, n):
    rr, ri = None, None
    while n:
        if n & 1:
            if rr is None:
                rr, ri = pr, pi
            else:
                rr, ri = rr * pr - ri * pi, rr * pi + ri * pr
        n >>= 1
        if n:
            pr, pi = pr * pr - pi * pi, 2.0 * pr * pi
    return rr, ri


def _kernel(x_hbm, lre_hbm, lim_hbm, ldt_hbm, dskip_hbm,
            bre_hbm, bim_hbm, cre_hbm, cim_hbm, wg_hbm, wu_hbm, wd_hbm,
            o_ref,
            lre_ref, lim_ref, ldt_ref, dskip_ref,
            bre_ref, bim_ref, cre_ref, cim_ref, wg_ref, wu_ref, wd_ref, sems, xsems,
            cst_ref, lam_ref, carry_ref, hin_ref, bu_ref, base_ref, a_ref, xbuf):
    P = bre_ref.shape[0]
    F = wg_ref.shape[0]
    f32 = jnp.float32
    bf16 = jnp.bfloat16
    NG = P // 128
    step_i = pl.program_id(0)
    nchunks = pl.num_programs(0) - 1
    nt = (((1,), (1,)), ((), ()))

    lo = lambda r: r.at[0:FSPLIT]
    hi = lambda r: r.at[FSPLIT:F]
    pairs = dict(lre=(lre_hbm, lre_ref), lim=(lim_hbm, lim_ref), ldt=(ldt_hbm, ldt_ref),
                 dskip=(dskip_hbm, dskip_ref),
                 bre=(bre_hbm, bre_ref), bim=(bim_hbm, bim_ref),
                 wg0=(lo(wg_hbm), lo(wg_ref)), wg1=(hi(wg_hbm), hi(wg_ref)),
                 wu0=(lo(wu_hbm), lo(wu_ref)), wu1=(hi(wu_hbm), hi(wu_ref)),
                 cre=(cre_hbm, cre_ref), cim=(cim_hbm, cim_ref),
                 wd=(wd_hbm, wd_ref))
    order = list(pairs)

    def copy(name):
        src, dst = pairs[name]
        return pltpu.make_async_copy(src, dst, sems.at[order.index(name)])

    def xcopy(c):
        slot = c % 2
        return pltpu.make_async_copy(x_hbm.at[pl.ds(c * TC, TC)], xbuf.at[slot], xsems.at[slot])

    def anycopy(n):
        return xcopy(int(n[1:])) if n.startswith('x') else copy(n)

    def start(*names):
        for n in names:
            anycopy(n).start()

    def wait(*names):
        for n in names:
            anycopy(n).wait()

    def init_small():
        lre = lre_ref[...].astype(f32).reshape(1, P)
        lim = lim_ref[...].astype(f32).reshape(1, P)
        ldt = ldt_ref[...].astype(f32).reshape(1, P)
        dt = jnp.exp(ldt).astype(bf16).astype(f32)
        e = jnp.exp(dt * lre)
        lbr = e * jnp.cos(dt * lim)
        lbi = e * jnp.sin(dt * lim)
        nr = lbr - 1.0
        ni = lbi
        den = lre * lre + lim * lim
        cr = (nr * lre + ni * lim) / den
        ci = (ni * lre - nr * lim) / den
        lam_ref[0:1, :] = lbr
        lam_ref[1:2, :] = lbi
        pr, pi = _cpow(lbr, lbi, SEG)
        lam_ref[2:3, :] = pr
        lam_ref[3:4, :] = pi
        pr, pi = _cpow(lbr, lbi, LAST)
        lam_ref[4:5, :] = pr
        lam_ref[5:6, :] = pi
        lam_ref[6:7, :] = cr
        lam_ref[7:8, :] = ci
        carry_ref[...] = jnp.zeros_like(carry_ref)
        for g in range(2 * NG):
            bu_ref[g, TC:NSEG * SEG, :] = jnp.zeros((NSEG * SEG - TC, 128), f32)

    def init_c():
        cr = lam_ref[6:7, :]
        ci = lam_ref[7:8, :]
        c_re = cre_ref[...].astype(f32)
        c_im = cim_ref[...].astype(f32)
        cst_ref[:, 0:P] = (2.0 * (c_re * cr - c_im * ci)).astype(bf16)
        cst_ref[:, P:2 * P] = (-2.0 * (c_re * ci + c_im * cr)).astype(bf16)

    def layernorm(ref):
        x = ref[...].astype(f32)
        m = jnp.mean(x, axis=-1, keepdims=True)
        xc = x - m
        v = jnp.mean(xc * xc, axis=-1, keepdims=True)
        return (xc * jax.lax.rsqrt(v + 1e-5)).astype(bf16)

    def project_re(xn):
        bu = jax.lax.dot_general(xn, bre_ref[...], nt, preferred_element_type=f32)
        for g in range(NG):
            bu_ref[g, 0:TC, :] = bu[:, g * 128:(g + 1) * 128]

    def project_im(xn):
        bu = jax.lax.dot_general(xn, bim_ref[...], nt, preferred_element_type=f32)
        for g in range(NG):
            bu_ref[NG + g, 0:TC, :] = bu[:, g * 128:(g + 1) * 128]

    def scan():
        lr = jnp.broadcast_to(lam_ref[0:1, :], (NSEG, P))
        li = jnp.broadcast_to(lam_ref[1:2, :], (NSEG, P))

        def step(j, h):
            hr, hi = h
            br = jnp.concatenate([bu_ref[g, pl.ds(j, NSEG, stride=SEG), :] for g in range(NG)], axis=1)
            bi = jnp.concatenate([bu_ref[NG + g, pl.ds(j, NSEG, stride=SEG), :] for g in range(NG)], axis=1)
            return lr * hr - li * hi + br, lr * hi + li * hr + bi

        z = jnp.zeros((NSEG, P), f32)
        fr, fi = jax.lax.fori_loop(0, LAST, step, (z, z), unroll=True)
        er, ei = jax.lax.fori_loop(LAST, SEG, step, (fr, fi), unroll=True)

        pr = lam_ref[2:3, :]
        pi = lam_ref[3:4, :]
        cr = carry_ref[0:1, :]
        ci = carry_ref[1:2, :]
        for s in range(NSEG):
            hin_ref[s:s + 1, 0:P] = cr
            hin_ref[s:s + 1, P:2 * P] = ci
            if s < NSEG - 1:
                cr, ci = (pr * cr - pi * ci + er[s:s + 1, :], pr * ci + pi * cr + ei[s:s + 1, :])
            else:
                pr = lam_ref[4:5, :]
                pi = lam_ref[5:6, :]
                cr, ci = (pr * cr - pi * ci + fr[s:s + 1, :], pr * ci + pi * cr + fi[s:s + 1, :])
        carry_ref[0:1, :] = cr
        carry_ref[1:2, :] = ci

        def step2(j, h):
            nr, ni = step(j, h)
            for g in range(NG):
                bu_ref[g, pl.ds(j, NSEG, stride=SEG), :] = nr[:, g * 128:(g + 1) * 128]
                bu_ref[NG + g, pl.ds(j, NSEG, stride=SEG), :] = ni[:, g * 128:(g + 1) * 128]
            return nr, ni

        h = jax.lax.fori_loop(0, LAST, step2, (hin_ref[:, 0:P], hin_ref[:, P:2 * P]), unroll=True)

        keep = jax.lax.broadcasted_iota(jnp.int32, (NSEG, P), 0) < NSEG - 1

        def step3(j, h):
            nr, ni = step(j, h)
            sr = jnp.where(keep, nr, 0.0)
            si = jnp.where(keep, ni, 0.0)
            for g in range(NG):
                bu_ref[g, pl.ds(j, NSEG, stride=SEG), :] = sr[:, g * 128:(g + 1) * 128]
                bu_ref[NG + g, pl.ds(j, NSEG, stride=SEG), :] = si[:, g * 128:(g + 1) * 128]
            return nr, ni

        jax.lax.fori_loop(LAST, SEG, step3, h, unroll=True)

    def project_c():
        hb = jnp.concatenate([bu_ref[g, 0:TC, :] for g in range(2 * NG)], axis=1).astype(bf16)
        return jax.lax.dot_general(hb, cst_ref[...], nt, preferred_element_type=f32)

    def gate_up(xn, a0, a1):
        g = jax.lax.dot_general(xn, wg_ref[a0:a1, :], nt, preferred_element_type=f32)
        u = jax.lax.dot_general(xn, wu_ref[a0:a1, :], nt, preferred_element_type=f32)
        return (jax.nn.gelu(g, approximate=True) * u).astype(bf16)

    def stash_base(x_cur, xn, y):
        base_ref[...] = (x_cur[...].astype(f32) + y
                         + xn.astype(f32) * dskip_ref[...].astype(f32).reshape(1, P))

    def finish_prev():
        o_ref[...] = base_ref[...] + jnp.dot(a_ref[...], wd_ref[...], preferred_element_type=f32)


    @pl.when(step_i == 0)
    def _first():
        start('x0', 'bre', 'lre', 'lim', 'ldt', 'dskip')
        wait('x0')
        start('bim')
        x_cur = xbuf.at[0]
        xn = layernorm(x_cur)
        wait('bre')
        start('wg0')
        project_re(xn)
        wait('bim')
        start('wu0')
        project_im(xn)
        wait('lre', 'lim', 'ldt', 'dskip')
        init_small()
        wait('wg0')
        start('wg1')
        g = jax.lax.dot_general(xn, wg_ref[0:FSPLIT, :], nt, preferred_element_type=f32)
        wait('wu0')
        start('wu1')
        u = jax.lax.dot_general(xn, wu_ref[0:FSPLIT, :], nt, preferred_element_type=f32)
        a_ref[:, 0:FSPLIT] = (jax.nn.gelu(g, approximate=True) * u).astype(bf16)
        wait('wg1')
        start('cre', 'cim')
        g = jax.lax.dot_general(xn, wg_ref[FSPLIT:F, :], nt, preferred_element_type=f32)
        wait('wu1')
        start('x1', 'wd')
        u = jax.lax.dot_general(xn, wu_ref[FSPLIT:F, :], nt, preferred_element_type=f32)
        a_ref[:, FSPLIT:F] = (jax.nn.gelu(g, approximate=True) * u).astype(bf16)
        scan()
        wait('cre', 'cim')
        init_c()
        stash_base(x_cur, xn, project_c())
        wait('wd')

    @pl.when(jnp.logical_and(step_i != 0, step_i != nchunks))
    def _steady():
        @pl.when(step_i + 1 < nchunks)
        def _():
            xcopy(step_i + 1).start()

        xcopy(step_i).wait()
        finish_prev()
        x_cur = xbuf.at[step_i % 2]
        xn = layernorm(x_cur)
        project_re(xn)
        project_im(xn)
        a = gate_up(xn, 0, F)
        scan()
        stash_base(x_cur, xn, project_c())
        a_ref[...] = a

    @pl.when(step_i == nchunks)
    def _last():
        finish_prev()


@jax.jit
def pallas_parallel_sum__ssm_conv_s5__geglu_ffn__prompt_kernel(
    A_x, A_Lambda_re, A_Lambda_im, A_B_re, A_B_im, A_C_re, A_C_im, A_log_dt, A_Dskip,
    B_x, B_w_gate, B_w_up, B_w_down,
):
    Bsz, L, D = A_x.shape
    P = A_Lambda_re.shape[0]
    F = B_w_gate.shape[1]
    x = A_x.reshape(L, D)
    hbm = pl.BlockSpec(memory_space=pl.ANY)
    out = pl.pallas_call(
        _kernel,
        grid=(L // TC + 1,),
        in_specs=[hbm] * 12,
        out_specs=pl.BlockSpec((TC, D), lambda i: (jnp.maximum(i - 1, 0), 0)),
        out_shape=jax.ShapeDtypeStruct((L, D), jnp.float32),
        scratch_shapes=[
            pltpu.VMEM((P,), jnp.bfloat16), pltpu.VMEM((P,), jnp.bfloat16),
            pltpu.VMEM((P,), jnp.bfloat16), pltpu.VMEM((D,), jnp.bfloat16),
            pltpu.VMEM((P, D), jnp.bfloat16), pltpu.VMEM((P, D), jnp.bfloat16),
            pltpu.VMEM((D, P), jnp.bfloat16), pltpu.VMEM((D, P), jnp.bfloat16),
            pltpu.VMEM((F, D), jnp.bfloat16), pltpu.VMEM((F, D), jnp.bfloat16),
            pltpu.VMEM((F, D), jnp.bfloat16),
            pltpu.SemaphoreType.DMA((13,)),
            pltpu.SemaphoreType.DMA((2,)),
            pltpu.VMEM((D, 2 * P), jnp.bfloat16),
            pltpu.VMEM((8, P), jnp.float32),
            pltpu.VMEM((8, P), jnp.float32),
            pltpu.VMEM((NSEG, 2 * P), jnp.float32),
            pltpu.VMEM((2 * P // 128, NSEG * SEG, 128), jnp.float32),
            pltpu.VMEM((TC, D), jnp.float32),
            pltpu.VMEM((TC, F), jnp.bfloat16),
            pltpu.VMEM((2, TC, D), jnp.bfloat16),
        ],
        compiler_params=pltpu.CompilerParams(
            dimension_semantics=("arbitrary",),
            vmem_limit_bytes=96 * 1024 * 1024,
        ),
    )(x, A_Lambda_re, A_Lambda_im, A_log_dt, A_Dskip,
      A_B_re, A_B_im, A_C_re, A_C_im, B_w_gate.T, B_w_up.T, B_w_down)
    return out.reshape(Bsz, L, D)
```
